```python
import jax
import jax.numpy as jnp

def _softmax(x, axis=-1):
    return jax.nn.softmax(x, axis=axis)
def _gelu(x):
    return jax.nn.gelu(x, approximate=True)
def _silu(x):
    return jax.nn.silu(x)
def _sigmoid(x):
    return jax.nn.sigmoid(x)
def _layernorm(x, axis=-1, eps=1e-5):
    m = jnp.mean(x, axis=axis, keepdims=True)
    v = jnp.var(x, axis=axis, keepdims=True)
    return (x - m) / jnp.sqrt(v + eps)
def _scatter_add(tgt, idx, src, axis=0):
    return tgt.at[idx].add(src)
def _segment_sum(src, seg, n):
    return jax.ops.segment_sum(src, seg, n)
class _Rng:
    def __init__(self, key):
        self._k = key
    def _next(self):
        self._k, sub = jax.random.split(self._k)
        return sub
    def normal(self, shape):
        return jax.random.normal(self._next(), shape, dtype=jnp.bfloat16)
    def randint(self, lo, hi, shape):
        return jax.random.randint(self._next(), shape, lo, hi, dtype=jnp.int32)
    def uniform(self, shape, lo=0.0, hi=1.0):
        return jax.random.uniform(self._next(), shape, jnp.bfloat16, lo, hi)
    def permutation(self, n):
        return jax.random.permutation(self._next(), n)


kernel_name = 'recurrent_scan__compressed_kv_cla__dense_activation_gelu__decode'

def setup_inputs():
    _rng = _Rng(jax.random.key(int.from_bytes(__import__("os").urandom(4), "little")))
    _w = (lambda a: (lambda t: t.astype(jnp.bfloat16) if jnp.issubdtype(t.dtype, jnp.floating) else t)(jnp.asarray(a)))
    def _A_setup():
        B, H, Sq, Sk, D, M = 2, 32, 1, 16384, 128, 512
        Dc = 4 * D
        return {
            "x": _w((lambda *s: _rng.normal(s) * 0.05)(B, Sq, M)),
            "c_kv": _w((lambda *s: _rng.normal(s) * 0.05)(B, Sk, Dc)),
            "w_q": _w((lambda *s: _rng.normal(s) * 0.05)(M, H, D) * (M ** -0.5)),
            "w_uk": _w((lambda *s: _rng.normal(s) * 0.05)(Dc, H, D) * (Dc ** -0.5)),
            "w_uv": _w((lambda *s: _rng.normal(s) * 0.05)(Dc, H, D) * (Dc ** -0.5)),
            "w_o": _w((lambda *s: _rng.normal(s) * 0.05)(H, D, M) * ((H * D) ** -0.5)),
        }
    _A_in = _A_setup()

    def _B_setup():
        B, S, D, F = 2, 1, 512, 1792
        return {
            "x": _w((lambda *s: _rng.normal(s) * 0.05)(B, S, D)),
            "w1": _w((lambda *s: _rng.normal(s) * 0.05)(D, F) * (D ** -0.5)),
            "b1": _w((lambda *s: _rng.normal(s) * 0.05)(F) * 0.01),
            "w2": _w((lambda *s: _rng.normal(s) * 0.05)(F, D) * (F ** -0.5)),
            "b2": _w((lambda *s: _rng.normal(s) * 0.05)(D) * 0.01),
        }
    _B_in = _B_setup()

    return {
        "A_x": _A_in["x"],
        "A_c_kv": _A_in["c_kv"],
        "A_w_q": _A_in["w_q"],
        "A_w_uk": _A_in["w_uk"],
        "A_w_uv": _A_in["w_uv"],
        "A_w_o": _A_in["w_o"],
        "B_x": _B_in["x"],
        "B_w1": _B_in["w1"],
        "B_b1": _B_in["b1"],
        "B_w2": _B_in["w2"],
        "B_b2": _B_in["b2"],
    }

def reference(A_x, A_c_kv, A_w_q, A_w_uk, A_w_uv, A_w_o, B_x, B_w1, B_b1, B_w2, B_b2):
    def _A_ref(x, c_kv, w_q, w_uk, w_uv, w_o):
        B, Sq, M = x.shape[0], x.shape[1], x.shape[2]
        Sk = c_kv.shape[1]
        H, D = w_q.shape[1], w_q.shape[2]
        q = jnp.einsum("bqm,mhd->bhqd", x, w_q)
        k = jnp.einsum("bkc,chd->bhkd", c_kv, w_uk)
        v = jnp.einsum("bkc,chd->bhkd", c_kv, w_uv)
        scores = jnp.einsum("bhqd,bhkd->bhqk", q, k) * (D ** -0.5)
        off = Sk - Sq
        qi = jnp.arange(Sq)[:, None]
        kj = jnp.arange(Sk)[None, :]
        cmask = kj <= (qi + off)
        scores = jnp.where(cmask[None, None], scores, -1e9)
        p = _softmax(scores, axis=-1)
        ctx = jnp.einsum("bhqk,bhkd->bhqd", p, v)
        return jnp.einsum("bhqd,hdm->bqm", ctx, w_o)

    def _B_ref(x, w1, b1, w2, b2):
        h = jnp.einsum("bsd,df->bsf", x, w1) + b1
        h = _gelu(h)
        return jnp.einsum("bsf,fd->bsd", h, w2) + b2

    x = A_x
    xn = _layernorm(x, axis=-1)
    s = _A_ref(xn, A_c_kv, A_w_q, A_w_uk, A_w_uv, A_w_o)
    g = _silu(_B_ref(xn, B_w1, B_b1, B_w2, B_b2))
    return x + s * g
```

```python
import functools

import jax
import jax.numpy as jnp
import jax.experimental.pallas as pl
import jax.experimental.pallas.tpu as pltpu
from jax import lax

_B, _H, _D, _M, _SK, _DC, _F = 2, 32, 128, 512, 16384, 512, 1792
_R = _B * _H
_BK = 1024
_NK = _SK // _BK
_NWC = 4
_WROWS = _M * _H // _NWC

_NT = (((1,), (1,)), ((), ()))


def _dot(a, b):
    return jnp.dot(a, b, preferred_element_type=jnp.float32)


def _dot_nt(a, b):
    return lax.dot_general(a, b, _NT, preferred_element_type=jnp.float32)


def _kernel(x_hbm, ckv_hbm, wq_hbm, wuk_hbm, wuv_hbm, wo_hbm, w1_hbm, b1_hbm, w2_hbm, b2_hbm,
            out_ref,
            x_v, b1_v, b2_v, ckv_v, wq_v, wuk_v, wuv_v, wo_v, w1_v, w2_v, l_v, et_v,
            sem_small, sem_w, sem_kv):
    f32, bf16 = jnp.float32, jnp.bfloat16

    cp_x = pltpu.make_async_copy(x_hbm, x_v, sem_small.at[0])
    cp_b1 = pltpu.make_async_copy(b1_hbm, b1_v, sem_small.at[1])
    cp_b2 = pltpu.make_async_copy(b2_hbm, b2_v, sem_small.at[2])

    def wchunks(src, dst, base):
        rows = src.shape[0] // _NWC
        return [pltpu.make_async_copy(src.at[pl.ds(i * rows, rows)], dst.at[pl.ds(i * rows, rows)],
                                      sem_w.at[base + i]) for i in range(_NWC)]

    cp_wq = wchunks(wq_hbm, wq_v, 0)
    cp_wuk = wchunks(wuk_hbm, wuk_v, _NWC)
    cp_wuv = wchunks(wuv_hbm, wuv_v, 2 * _NWC)
    cp_wo = wchunks(wo_hbm, wo_v, 3 * _NWC)
    cp_w1 = pltpu.make_async_copy(w1_hbm, w1_v, sem_w.at[4 * _NWC])
    cp_w2 = pltpu.make_async_copy(w2_hbm, w2_v, sem_w.at[4 * _NWC + 1])

    def cp_kv(b, i):
        rows = pl.ds(pl.multiple_of(i * _BK, _BK), _BK)
        return pltpu.make_async_copy(ckv_hbm.at[b, rows], ckv_v.at[b, rows], sem_kv.at[i * _B + b])

    cp_x.start()
    for c in cp_wq + cp_wuk:
        c.start()
    cp_b1.start()
    cp_b2.start()
    for i in range(_NK):
        for b in range(_B):
            cp_kv(b, i).start()
        if i == 1:
            cp_w1.start()
            cp_w2.start()
    for c in cp_wuv + cp_wo:
        c.start()

    r = lax.broadcasted_iota(jnp.int32, (_WROWS, 128), 0)
    c_ = lax.broadcasted_iota(jnp.int32, (_WROWS, 128), 1)
    et_v[...] = (r // _H == c_).astype(f32).astype(bf16)

    row_h = lax.broadcasted_iota(jnp.int32, (_R, 128), 0) % _H
    lane = lax.broadcasted_iota(jnp.int32, (_R, 128), 1)
    diag = row_h == (lane % _H)

    cp_x.wait()
    x = jnp.concatenate([x_v[0], x_v[1]], axis=0).astype(f32)
    mu = jnp.mean(x, axis=-1, keepdims=True)
    xc = x - mu
    var = jnp.mean(xc * xc, axis=-1, keepdims=True)
    xn = (xc / jnp.sqrt(var + 1e-5)).astype(bf16)

    t_ = lax.broadcasted_iota(jnp.int32, (128, _M), 0)
    m_ = lax.broadcasted_iota(jnp.int32, (128, _M), 1)
    sel_t = (m_ // 4) == t_
    mm = lax.broadcasted_iota(jnp.int32, (_M, 128), 0)
    ll = lax.broadcasted_iota(jnp.int32, (_M, 128), 1)
    fmat = ((ll // _H) == (mm % 4)).astype(f32).astype(bf16)
    xe = []
    for b in range(_B):
        a = jnp.where(sel_t, jnp.broadcast_to(xn[b:b + 1, :].astype(f32), (128, _M)), 0.0).astype(bf16)
        xe.append(_dot(a, fmat))
    for t in range(128):
        rows = jnp.concatenate(
            [jnp.broadcast_to(xe[b][t:t + 1, :], (_H, 128)) for b in range(_B)], axis=0)
        l_v[:, t * 128:(t + 1) * 128] = jnp.where(diag, rows, 0.0).astype(bf16)

    q = jnp.zeros((_R, _D), f32)
    for i in range(_NWC):
        cp_wq[i].wait()
        q = q + _dot(l_v[:, i * _WROWS:(i + 1) * _WROWS], wq_v[i * _WROWS:(i + 1) * _WROWS, :])
    q = q.astype(bf16)

    diag_w = jnp.concatenate([diag] * (_WROWS // 128), axis=1)
    scale = _D ** -0.5
    qa = []
    for i in range(_NWC):
        cp_wuk[i].wait()
        full = _dot_nt(q, wuk_v[i * _WROWS:(i + 1) * _WROWS, :])
        msk = jnp.where(diag_w, full * scale, 0.0).astype(bf16)
        qa.append(_dot(msk, et_v[...]).astype(bf16))
    qabs = jnp.concatenate(qa, axis=1)
    qb = [qabs[b * _H:(b + 1) * _H, :] for b in range(_B)]

    cp_w1.wait()
    cp_b1.wait()
    hpre = _dot(xn, w1_v[...]) + b1_v[...].reshape(1, _F).astype(f32)
    hact = jax.nn.gelu(hpre, approximate=True).astype(bf16)
    cp_w2.wait()
    cp_b2.wait()
    y = _dot(hact, w2_v[...]) + b2_v[...].reshape(1, _M).astype(f32)
    g = y * jax.nn.sigmoid(y)

    def body(i, carry):
        new = []
        for b in range(_B):
            m_prev, l_prev, acc = carry[b]
            cp_kv(b, i).wait()
            kv = ckv_v[b, pl.ds(pl.multiple_of(i * _BK, _BK), _BK), :]
            s = _dot_nt(qb[b], kv)
            m_new = jnp.maximum(m_prev, jnp.max(s, axis=-1, keepdims=True))
            alpha = jnp.exp(m_prev - m_new)
            p = jnp.exp(s - m_new)
            l_new = alpha * l_prev + jnp.sum(p, axis=-1, keepdims=True)
            acc = alpha * acc + _dot(p.astype(bf16), kv)
            new.append((m_new, l_new, acc))
        return tuple(new)

    init = tuple((jnp.full((_H, 1), -jnp.inf, f32), jnp.zeros((_H, 1), f32),
                  jnp.zeros((_H, _DC), f32)) for _ in range(_B))
    res = lax.fori_loop(0, _NK, body, init)
    ctxc = jnp.concatenate([res[b][2] / res[b][1] for b in range(_B)], axis=0).astype(bf16)

    ctx = jnp.zeros((_R, _D), f32)
    for i in range(_NWC):
        expd = _dot_nt(ctxc[:, i * 128:(i + 1) * 128], et_v[...])
        lv = jnp.where(diag_w, expd, 0.0).astype(bf16)
        cp_wuv[i].wait()
        ctx = ctx + _dot(lv, wuv_v[i * _WROWS:(i + 1) * _WROWS, :])
    ctx = ctx.astype(bf16).astype(f32)

    sacc = jnp.zeros((_R, _M), f32)
    hpc = _H // _NWC
    for i in range(_NWC):
        cp_wo[i].wait()
        for hh in range(hpc):
            h = i * hpc + hh
            lh = jnp.where(row_h == h, ctx, 0.0).astype(bf16)
            sacc = sacc + _dot(lh, wo_v[h * _D:(h + 1) * _D, :])
    s_out = jnp.concatenate(
        [jnp.sum(sacc[b * _H:(b + 1) * _H], axis=0, keepdims=True) for b in range(_B)], axis=0)

    o = (x + s_out * g).astype(out_ref.dtype)
    for b in range(_B):
        out_ref[b] = o[b:b + 1, :]


@jax.jit
def pallas_recurrent_scan__compressed_kv_cla__dense_activation_gelu__decode_kernel(
    A_x: jax.Array,
    A_c_kv: jax.Array,
    A_w_q: jax.Array,
    A_w_uk: jax.Array,
    A_w_uv: jax.Array,
    A_w_o: jax.Array,
    B_x: jax.Array,
    B_w1: jax.Array,
    B_b1: jax.Array,
    B_w2: jax.Array,
    B_b2: jax.Array,
):
    del B_x
    bf16 = jnp.bfloat16
    hbm = pl.BlockSpec(memory_space=pl.ANY)
    scratch = [
        pltpu.VMEM((_B, 1, _M), bf16),
        pltpu.VMEM((_F,), bf16),
        pltpu.VMEM((_M,), bf16),
        pltpu.VMEM((_B, _SK, _DC), bf16),
        pltpu.VMEM((_M * _H, _D), bf16),
        pltpu.VMEM((_DC * _H, _D), bf16),
        pltpu.VMEM((_DC * _H, _D), bf16),
        pltpu.VMEM((_H * _D, _M), bf16),
        pltpu.VMEM((_M, _F), bf16),
        pltpu.VMEM((_F, _M), bf16),
        pltpu.VMEM((_R, _M * _H), bf16),
        pltpu.VMEM((_WROWS, 128), bf16),
        pltpu.SemaphoreType.DMA((3,)),
        pltpu.SemaphoreType.DMA((4 * _NWC + 2,)),
        pltpu.SemaphoreType.DMA((_NK * _B,)),
    ]
    return pl.pallas_call(
        _kernel,
        out_shape=jax.ShapeDtypeStruct(A_x.shape, A_x.dtype),
        in_specs=[hbm] * 10,
        out_specs=pl.BlockSpec(memory_space=pltpu.VMEM),
        scratch_shapes=scratch,
        compiler_params=pltpu.CompilerParams(vmem_limit_bytes=100 * 1024 * 1024),
    )(A_x, A_c_kv, A_w_q.reshape(_M * _H, _D), A_w_uk.reshape(_DC * _H, _D),
      A_w_uv.reshape(_DC * _H, _D), A_w_o.reshape(_H * _D, _M), B_w1, B_b1, B_w2, B_b2)
```

```python
import functools

import jax
import jax.numpy as jnp
import jax.experimental.pallas as pl
import jax.experimental.pallas.tpu as pltpu
from jax import lax

_B, _H, _D, _M, _SK, _DC, _F = 2, 32, 128, 512, 16384, 512, 1792
_R = _B * _H
_BK = 1024
_NK = _SK // _BK
_NS = _DC // 128
_NWC = 4
_WROWS = _M * _H // _NWC
_NWO = 8
PROF = False

_NT = (((1,), (1,)), ((), ()))


def _dot(a, b):
    return jnp.dot(a, b, preferred_element_type=jnp.float32)


def _dot_nt(a, b):
    return lax.dot_general(a, b, _NT, preferred_element_type=jnp.float32)


def _kernel(x_hbm, ckv_hbm, wq_hbm, wuk_hbm, wuv_hbm, wo_hbm, w1_hbm, b1_hbm, w2_hbm, b2_hbm,
            out_ref,
            x_v, b1_v, b2_v, ckv_v, wq_v, wuk_v, wuv_v, wo_v, w1_v, w2_v, l_v, et_v,
            sem_small, sem_wq, sem_wuk, sem_wuv, sem_wo, sem_mlp, sem_kv):
    f32, bf16 = jnp.float32, jnp.bfloat16
    sc = jax.named_scope

    cp_x = pltpu.make_async_copy(x_hbm, x_v, sem_small.at[0])
    cp_b1 = pltpu.make_async_copy(b1_hbm, b1_v, sem_small.at[1])
    cp_b2 = pltpu.make_async_copy(b2_hbm, b2_v, sem_small.at[2])

    def half(src, dst, sem):
        def f(i):
            rows = src.shape[0] // 2
            r = pl.ds(pl.multiple_of(i * rows, rows), rows)
            return pltpu.make_async_copy(src.at[r], dst.at[r], sem.at[i])
        return f

    cp_wq = half(wq_hbm, wq_v, sem_wq)
    cp_wuk = half(wuk_hbm, wuk_v, sem_wuk)
    cp_wuv = half(wuv_hbm, wuv_v, sem_wuv)
    cp_w1 = pltpu.make_async_copy(w1_hbm, w1_v, sem_mlp.at[0])
    cp_w2 = pltpu.make_async_copy(w2_hbm, w2_v, sem_mlp.at[1])

    def cp_wo(i):
        rows = _H * _D // _NWO
        r = pl.ds(pl.multiple_of(i * rows, rows), rows)
        return [pltpu.make_async_copy(wo_hbm.at[r, pl.ds(j * 128, 128)], wo_v.at[j, r], sem_wo.at[i])
                for j in range(_M // 128)]

    def cp_kv(i):
        r = pl.ds(pl.multiple_of(i * _BK, _BK), _BK)
        return [pltpu.make_async_copy(ckv_hbm.at[:, r, pl.ds(j * 128, 128)], ckv_v.at[:, j, r],
                                      sem_kv.at[i]) for j in range(_NS)]

    def issue(n, f):
        def body(i, _):
            d = f(i)
            for c in (d if isinstance(d, (list, tuple)) else [d]):
                c.start()
        lax.fori_loop(0, n, body, None)

    with sc("issue"):
        cp_x.start()
        cp_b1.start()
        cp_b2.start()
        issue(2, cp_wq)
        issue(2, cp_wuk)
        issue(_NK, cp_kv)

        def mlp_i(i, _):
            pl.when(i == 0)(lambda: cp_w1.start())
            pl.when(i == 1)(lambda: cp_w2.start())
        lax.fori_loop(0, 2, mlp_i, None)
        issue(2, cp_wuv)
        issue(_NWO, cp_wo)

    with sc("const"):
        r = lax.broadcasted_iota(jnp.int32, (_WROWS, 128), 0)
        c_ = lax.broadcasted_iota(jnp.int32, (_WROWS, 128), 1)
        et_v[...] = (r // _H == c_).astype(f32).astype(bf16)

        row_h = lax.broadcasted_iota(jnp.int32, (_R, 128), 0) % _H
        lane = lax.broadcasted_iota(jnp.int32, (_R, 128), 1)
        diag = row_h == (lane % _H)

    with sc("ln"):
        cp_x.wait()
        x = x_v[...].astype(f32)
        mu = jnp.mean(x, axis=-1, keepdims=True)
        xc = x - mu
        var = jnp.mean(xc * xc, axis=-1, keepdims=True)
        xn = (xc / jnp.sqrt(var + 1e-5)).astype(bf16)

        t_ = lax.broadcasted_iota(jnp.int32, (128, _M), 0)
        m_ = lax.broadcasted_iota(jnp.int32, (128, _M), 1)
        sel_t = (m_ // 4) == t_
        mm = lax.broadcasted_iota(jnp.int32, (_M, 128), 0)
        ll = lax.broadcasted_iota(jnp.int32, (_M, 128), 1)
        fmat = ((ll // _H) == (mm % 4)).astype(f32).astype(bf16)
        xe = []
        for b in range(_B):
            a = jnp.where(sel_t, jnp.broadcast_to(xn[b:b + 1, :].astype(f32), (128, _M)), 0.0).astype(bf16)
            xe.append(_dot(a, fmat))
        for t in range(128):
            rows = jnp.concatenate(
                [jnp.broadcast_to(xe[b][t:t + 1, :], (_H, 128)) for b in range(_B)], axis=0)
            l_v[:, t * 128:(t + 1) * 128] = jnp.where(diag, rows, 0.0).astype(bf16)

    with sc("q"):
        q = jnp.zeros((_R, _D), f32)
        for i in range(_NWC):
            if i % 2 == 0:
                cp_wq(i // 2).wait()
            q = q + _dot(l_v[:, i * _WROWS:(i + 1) * _WROWS], wq_v[i * _WROWS:(i + 1) * _WROWS, :])
        q = q.astype(bf16)

    with sc("qabs"):
        diag_w = jnp.concatenate([diag] * (_WROWS // 128), axis=1)
        scale = _D ** -0.5
        qa = []
        for i in range(_NWC):
            if i % 2 == 0:
                cp_wuk(i // 2).wait()
            full = _dot_nt(q, wuk_v[i * _WROWS:(i + 1) * _WROWS, :])
            msk = jnp.where(diag_w, full * scale, 0.0).astype(bf16)
            qa.append(_dot(msk, et_v[...]).astype(bf16))

    with sc("attn"):
        def body(i, carry):
            for c in cp_kv(i):
                c.wait()
            rows = pl.ds(pl.multiple_of(i * _BK, _BK), _BK)
            new = []
            for b in range(_B):
                m_prev, l_prev, acc = carry[b]
                s = None
                for j in range(_NS):
                    sj = _dot_nt(qa[j][b * _H:(b + 1) * _H, :], ckv_v[b, j, rows, :])
                    s = sj if s is None else s + sj
                m_new = jnp.maximum(m_prev, jnp.max(s, axis=-1, keepdims=True))
                alpha = jnp.exp(m_prev - m_new)
                p = jnp.exp(s - m_new)
                l_new = alpha * l_prev + jnp.sum(p, axis=-1, keepdims=True)
                pb = p.astype(bf16)
                acc = [alpha * acc[j] + _dot(pb, ckv_v[b, j, rows, :]) for j in range(_NS)]
                new.append((m_new, l_new, acc))
            return tuple(new)

        init = tuple((jnp.full((_H, 1), -jnp.inf, f32), jnp.zeros((_H, 1), f32),
                      [jnp.zeros((_H, 128), f32) for _ in range(_NS)]) for _ in range(_B))
        res = lax.fori_loop(0, _NK, body, init)
        ctxc = [jnp.concatenate([res[b][2][j] / res[b][1] for b in range(_B)], axis=0).astype(bf16)
                for j in range(_NS)]

    with sc("mlp"):
        cp_w1.wait()
        cp_b1.wait()
        hpre = _dot(xn, w1_v[...]) + b1_v[...].reshape(1, _F).astype(f32)
        hact = jax.nn.gelu(hpre, approximate=True).astype(bf16)
        cp_w2.wait()
        cp_b2.wait()
        y = _dot(hact, w2_v[...]) + b2_v[...].reshape(1, _M).astype(f32)
        g = y * jax.nn.sigmoid(y)

    with sc("ctx"):
        ctx = jnp.zeros((_R, _D), f32)
        for i in range(_NWC):
            expd = _dot_nt(ctxc[i], et_v[...])
            lv = jnp.where(diag_w, expd, 0.0).astype(bf16)
            if i % 2 == 0:
                cp_wuv(i // 2).wait()
            ctx = ctx + _dot(lv, wuv_v[i * _WROWS:(i + 1) * _WROWS, :])
        ctx = ctx.astype(bf16).astype(f32)

    with sc("out"):
        sacc = [jnp.zeros((_R, 128), f32) for _ in range(4)]
        hpc = _H // _NWO
        for i in range(_NWO):
            for c in cp_wo(i):
                c.wait()
            for hh in range(hpc):
                h = i * hpc + hh
                lh = jnp.where(row_h == h, ctx, 0.0).astype(bf16)
                for j in range(4):
                    sacc[j] = sacc[j] + _dot(lh, wo_v[j, h * _D:(h + 1) * _D, :])
        sacc = jnp.concatenate(sacc, axis=1)
        s_out = jnp.concatenate(
            [jnp.sum(sacc[b * _H:(b + 1) * _H], axis=0, keepdims=True) for b in range(_B)], axis=0)

        out_ref[...] = (x + s_out * g).astype(out_ref.dtype)


@jax.jit
def pallas_recurrent_scan__compressed_kv_cla__dense_activation_gelu__decode_kernel(
    A_x, A_c_kv, A_w_q, A_w_uk, A_w_uv, A_w_o, B_x, B_w1, B_b1, B_w2, B_b2,
):
    del B_x
    bf16 = jnp.bfloat16
    hbm = pl.BlockSpec(memory_space=pl.ANY)
    dma = pltpu.SemaphoreType.DMA
    scratch = [
        pltpu.VMEM((_B, _M), bf16),
        pltpu.VMEM((_F,), bf16),
        pltpu.VMEM((_M,), bf16),
        pltpu.VMEM((_B, _NS, _SK, 128), bf16),
        pltpu.VMEM((_M * _H, _D), bf16),
        pltpu.VMEM((_DC * _H, _D), bf16),
        pltpu.VMEM((_DC * _H, _D), bf16),
        pltpu.VMEM((4, _H * _D, 128), bf16),
        pltpu.VMEM((_M, _F), bf16),
        pltpu.VMEM((_F, _M), bf16),
        pltpu.VMEM((_R, _M * _H), bf16),
        pltpu.VMEM((_WROWS, 128), bf16),
        dma((3,)), dma((2,)), dma((2,)), dma((2,)), dma((_NWO,)), dma((2,)), dma((_NK,)),
    ]
    out = pl.pallas_call(
        _kernel,
        out_shape=jax.ShapeDtypeStruct((_B, _M), A_x.dtype),
        in_specs=[hbm] * 10,
        out_specs=pl.BlockSpec(memory_space=pltpu.VMEM),
        scratch_shapes=scratch,
        compiler_params=pltpu.CompilerParams(vmem_limit_bytes=100 * 1024 * 1024),
    )(A_x.reshape(_B, _M), A_c_kv, A_w_q.reshape(_M * _H, _D), A_w_uk.reshape(_DC * _H, _D),
      A_w_uv.reshape(_DC * _H, _D), A_w_o.reshape(_H * _D, _M), B_w1, B_b1, B_w2, B_b2)
    return out.reshape(A_x.shape)
```

```python
import jax
import jax.experimental.pallas as pl
import jax.experimental.pallas.tpu as pltpu
import jax.numpy as jnp
from jax import lax

_B, _H, _D, _M, _SK, _DC, _F = 2, 32, 128, 512, 16384, 512, 1792
_R = _B * _H
_BK = 4096
_NK = _SK // _BK
_NS = _DC // 128
_NWC = 4
_WROWS = _M * _H // _NWC
_WO_HEADS = (16, 10, 4, 2)
_NWO = len(_WO_HEADS)
_WO_OFF = tuple(sum(_WO_HEADS[:i]) for i in range(_NWO + 1))

_NT = (((1,), (1,)), ((), ()))


def _dot(a, b):
    return jnp.dot(a, b, preferred_element_type=jnp.float32)


def _dot_nt(a, b):
    return lax.dot_general(a, b, _NT, preferred_element_type=jnp.float32)


def _kernel(x_hbm, ckv_hbm, wq_hbm, wuk_hbm, wuv_hbm, wo_hbm, w1_hbm, b1_hbm, w2_hbm, b2_hbm,
            out_ref,
            x_v, b1_v, b2_v, ckv_v, wq_v, wuk_v, wuv_v, wo_v, w1_v, w2_v, l_v, et_v, sem):
    f32, bf16 = jnp.float32, jnp.bfloat16

    def copy(src, dst, slot):
        return pltpu.make_async_copy(src, dst, sem.at[slot])

    cp_small = [copy(x_hbm, x_v, 0), copy(b1_hbm, b1_v, 0), copy(b2_hbm, b2_v, 0)]
    cp_wq = copy(wq_hbm, wq_v, 1)
    cp_wuk = copy(wuk_hbm, wuk_v, 2)
    cp_mlp = [copy(w1_hbm, w1_v, 3), copy(w2_hbm, w2_v, 3)]
    cp_wuv = copy(wuv_hbm, wuv_v, 4)

    def cp_wo(i):
        r = pl.ds(_WO_OFF[i] * _D, _WO_HEADS[i] * _D)
        return copy(wo_hbm.at[r], wo_v.at[r], 5 + i)

    def cp_kv(i):
        r = pl.ds(pl.multiple_of(i * _BK, _BK), _BK)
        return [copy(ckv_hbm.at[:, r, pl.ds(j * 128, 128)], ckv_v.at[:, j, r], 5 + _NWO + i)
                for j in range(_NS)]

    def in_order(groups):
        def body(i, _):
            for k, grp in enumerate(groups):
                @pl.when(i == k)
                def _(grp=grp):
                    for c in grp:
                        c.start()
        lax.fori_loop(0, len(groups), body, None)

    for c in cp_small:
        c.start()
    in_order([[cp_wq], [cp_wuk]])

    def kv_start(i, _):
        for c in cp_kv(i):
            c.start()
    lax.fori_loop(0, _NK, kv_start, None)
    in_order([cp_mlp, [cp_wuv]] + [[cp_wo(i)] for i in range(_NWO)])

    r_ = lax.broadcasted_iota(jnp.int32, (_WROWS, 128), 0)
    c_ = lax.broadcasted_iota(jnp.int32, (_WROWS, 128), 1)
    et_v[...] = (r_ // _H == c_).astype(f32).astype(bf16)

    row_h = lax.broadcasted_iota(jnp.int32, (_R, 128), 0) % _H
    lane = lax.broadcasted_iota(jnp.int32, (_R, 128), 1)
    diag = row_h == (lane % _H)
    diag_w = jnp.concatenate([diag] * (_WROWS // 128), axis=1)

    for c in cp_small:
        c.wait()
    x = x_v[...].astype(f32)
    mu = jnp.mean(x, axis=-1, keepdims=True)
    xc = x - mu
    var = jnp.mean(xc * xc, axis=-1, keepdims=True)
    xn = (xc / jnp.sqrt(var + 1e-5)).astype(bf16)

    t_ = lax.broadcasted_iota(jnp.int32, (128, _M), 0)
    m_ = lax.broadcasted_iota(jnp.int32, (128, _M), 1)
    sel_t = (m_ // 4) == t_
    mm = lax.broadcasted_iota(jnp.int32, (_M, 128), 0)
    ll = lax.broadcasted_iota(jnp.int32, (_M, 128), 1)
    fmat = ((ll // _H) == (mm % 4)).astype(f32).astype(bf16)
    xe = []
    for b in range(_B):
        a = jnp.where(sel_t, jnp.broadcast_to(xn[b:b + 1, :].astype(f32), (128, _M)), 0.0)
        xe.append(_dot(a.astype(bf16), fmat))
    for t in range(128):
        rows = jnp.concatenate(
            [jnp.broadcast_to(xe[b][t:t + 1, :], (_H, 128)) for b in range(_B)], axis=0)
        l_v[:, t * 128:(t + 1) * 128] = jnp.where(diag, rows, 0.0).astype(bf16)

    cp_wq.wait()
    q = jnp.zeros((_R, _D), f32)
    for i in range(_NWC):
        q = q + _dot(l_v[:, i * _WROWS:(i + 1) * _WROWS], wq_v[i * _WROWS:(i + 1) * _WROWS, :])
    q = q.astype(bf16)

    cp_wuk.wait()
    scale = _D ** -0.5
    qa = []
    for i in range(_NWC):
        full = _dot_nt(q, wuk_v[i * _WROWS:(i + 1) * _WROWS, :])
        msk = jnp.where(diag_w, full * scale, 0.0).astype(bf16)
        qa.append(_dot(msk, et_v[...]).astype(bf16))

    def body(i, carry):
        for c in cp_kv(i):
            c.wait()
        rows = pl.ds(pl.multiple_of(i * _BK, _BK), _BK)
        new = []
        for b in range(_B):
            m_prev, l_prev, acc = carry[b]
            s = None
            for j in range(_NS):
                sj = _dot_nt(qa[j][b * _H:(b + 1) * _H, :], ckv_v[b, j, rows, :])
                s = sj if s is None else s + sj
            m_new = jnp.maximum(m_prev, jnp.max(s, axis=-1, keepdims=True))
            alpha = jnp.exp(m_prev - m_new)
            p = jnp.exp(s - m_new)
            l_new = alpha * l_prev + jnp.sum(p, axis=-1, keepdims=True)
            pb = p.astype(bf16)
            acc = [alpha * acc[j] + _dot(pb, ckv_v[b, j, rows, :]) for j in range(_NS)]
            new.append((m_new, l_new, acc))
        return tuple(new)

    init = tuple((jnp.full((_H, 1), -jnp.inf, f32), jnp.zeros((_H, 1), f32),
                  [jnp.zeros((_H, 128), f32) for _ in range(_NS)]) for _ in range(_B))
    res = lax.fori_loop(0, _NK, body, init)
    ctxc = [jnp.concatenate([res[b][2][j] / res[b][1] for b in range(_B)], axis=0).astype(bf16)
            for j in range(_NS)]

    for c in cp_mlp:
        c.wait()
    hpre = _dot(xn, w1_v[...]) + b1_v[...].reshape(1, _F).astype(f32)
    hact = jax.nn.gelu(hpre, approximate=True).astype(bf16)
    y = _dot(hact, w2_v[...]) + b2_v[...].reshape(1, _M).astype(f32)
    g = y * jax.nn.sigmoid(y)

    ctx = jnp.zeros((_R, _D), f32)
    for i in range(_NWC):
        expd = _dot_nt(ctxc[i], et_v[...])
        lv = jnp.where(diag_w, expd, 0.0).astype(bf16)
        if i == 0:
            cp_wuv.wait()
        ctx = ctx + _dot(lv, wuv_v[i * _WROWS:(i + 1) * _WROWS, :])

    ctx_h = [jnp.concatenate([ctx[b * _H + h:b * _H + h + 1, :] for b in range(_B)], axis=0).astype(bf16)
             for h in range(_H)]
    s_out = jnp.zeros((_B, _M), f32)
    for i in range(_NWO):
        lhs = jnp.concatenate(ctx_h[_WO_OFF[i]:_WO_OFF[i + 1]], axis=1)
        cp_wo(i).wait()
        s_out = s_out + _dot(lhs, wo_v[_WO_OFF[i] * _D:_WO_OFF[i + 1] * _D, :])
    out_ref[...] = (x + s_out * g).astype(out_ref.dtype)


@jax.jit
def pallas_recurrent_scan__compressed_kv_cla__dense_activation_gelu__decode_kernel(
    A_x: jax.Array,
    A_c_kv: jax.Array,
    A_w_q: jax.Array,
    A_w_uk: jax.Array,
    A_w_uv: jax.Array,
    A_w_o: jax.Array,
    B_x: jax.Array,
    B_w1: jax.Array,
    B_b1: jax.Array,
    B_w2: jax.Array,
    B_b2: jax.Array,
):
    del B_x
    bf16 = jnp.bfloat16
    hbm = pl.BlockSpec(memory_space=pl.ANY)
    scratch = [
        pltpu.VMEM((_B, _M), bf16),
        pltpu.VMEM((_F,), bf16),
        pltpu.VMEM((_M,), bf16),
        pltpu.VMEM((_B, _NS, _SK, 128), bf16),
        pltpu.VMEM((_M * _H, _D), bf16),
        pltpu.VMEM((_DC * _H, _D), bf16),
        pltpu.VMEM((_DC * _H, _D), bf16),
        pltpu.VMEM((_H * _D, _M), bf16),
        pltpu.VMEM((_M, _F), bf16),
        pltpu.VMEM((_F, _M), bf16),
        pltpu.VMEM((_R, _M * _H), bf16),
        pltpu.VMEM((_WROWS, 128), bf16),
        pltpu.SemaphoreType.DMA((5 + _NWO + _NK,)),
    ]
    out = pl.pallas_call(
        _kernel,
        out_shape=jax.ShapeDtypeStruct((_B, _M), A_x.dtype),
        in_specs=[hbm] * 10,
        out_specs=pl.BlockSpec(memory_space=pltpu.VMEM),
        scratch_shapes=scratch,
        compiler_params=pltpu.CompilerParams(vmem_limit_bytes=100 * 1024 * 1024),
    )(A_x.reshape(_B, _M), A_c_kv, A_w_q.reshape(_M * _H, _D), A_w_uk.reshape(_DC * _H, _D),
      A_w_uv.reshape(_DC * _H, _D), A_w_o.reshape(_H * _D, _M), B_w1, B_b1, B_w2, B_b2)
    return out.reshape(A_x.shape)
```
